```python
import jax
import jax.numpy as jnp

def _softmax(x, axis=-1):
    return jax.nn.softmax(x, axis=axis)
def _gelu(x):
    return jax.nn.gelu(x, approximate=True)
def _silu(x):
    return jax.nn.silu(x)
def _sigmoid(x):
    return jax.nn.sigmoid(x)
def _layernorm(x, axis=-1, eps=1e-5):
    m = jnp.mean(x, axis=axis, keepdims=True)
    v = jnp.var(x, axis=axis, keepdims=True)
    return (x - m) / jnp.sqrt(v + eps)
def _scatter_add(tgt, idx, src, axis=0):
    return tgt.at[idx].add(src)
def _segment_sum(src, seg, n):
    return jax.ops.segment_sum(src, seg, n)
class _Rng:
    def __init__(self, key):
        self._k = key
    def _next(self):
        self._k, sub = jax.random.split(self._k)
        return sub
    def normal(self, shape):
        return jax.random.normal(self._next(), shape, dtype=jnp.bfloat16)
    def randint(self, lo, hi, shape):
        return jax.random.randint(self._next(), shape, lo, hi, dtype=jnp.int32)
    def uniform(self, shape, lo=0.0, hi=1.0):
        return jax.random.uniform(self._next(), shape, jnp.bfloat16, lo, hi)
    def permutation(self, n):
        return jax.random.permutation(self._next(), n)


kernel_name = 'standalone__groupnorm__prompt'

def setup_inputs():
    _rng = _Rng(jax.random.key(int.from_bytes(__import__("os").urandom(4), "little")))
    _w = (lambda a: (lambda t: t.astype(jnp.bfloat16) if jnp.issubdtype(t.dtype, jnp.floating) else t)(jnp.asarray(a)))
    B = 2
    G = 32
    cpg = max(1, 1024 // G)
    C = G * cpg
    H, W = 32, 2048
    return {
        "x": _w((lambda *s: _rng.normal(s) * 0.05)(B, C, H, W)),
        "g": _w((lambda *s: _rng.normal(s) * 0.05)(C) + 1.0),
        "b": _w((lambda *s: _rng.normal(s) * 0.05)(C)),
    }

def reference(x, g, b):
    G = 32
    B, C, H, W = x.shape[0], x.shape[1], x.shape[2], x.shape[3]
    xr = x.reshape(B, G, C // G, H, W)
    mu = xr.mean(axis=(2, 3, 4), keepdims=True)
    var = ((xr - mu) ** 2).mean(axis=(2, 3, 4), keepdims=True)
    xn = (xr - mu) / jnp.sqrt(var + 1e-5)
    xn = xn.reshape(B, C, H, W)
    return xn * g[None, :, None, None] + b[None, :, None, None]
```

```python
import functools

import jax
import jax.numpy as jnp
from jax import lax
import jax.experimental.pallas as pl
import jax.experimental.pallas.tpu as pltpu

_GROUPS = 32
_EPS = 1e-5
_LANES = 128
_ROWS = 8
_SLAB = 32
_PHASE_GROUPS = 16
_READ_TAIL = 3
_WRITE_TAIL = 3


def _start(copies):
    for copy in copies:
        copy.start()


def _wait(copies):
    for copy in copies:
        copy.wait()


def _groupnorm_kernel(x_hbm, g_hbm, b_hbm, o_hbm, buf, gb_raw, gb_f32, gb,
                      read_sems, write_sems, param_sems, *, cpg, strips_per_ch):
    n = _PHASE_GROUPS
    width = buf.shape[-1]
    slabs = buf.shape[0] // n
    ch_per_slab = _SLAB // strips_per_ch
    phases = x_hbm.shape[0] // buf.shape[0]
    inv_count = 1.0 / (slabs * _SLAB * _ROWS * width)
    last = (n - 1) * slabs

    def read(phase, slot):
        return pltpu.make_async_copy(
            x_hbm.at[pl.ds((phase * n + slot) * slabs, slabs)],
            buf.at[pl.ds(slot * slabs, slabs)], read_sems.at[slot])

    def read_last(phase):
        def part(strips, sem):
            return pltpu.make_async_copy(
                x_hbm.at[pl.ds(phase * n * slabs + last, slabs), strips],
                buf.at[pl.ds(last, slabs), strips], sem)
        head = _SLAB - _READ_TAIL
        return (part(pl.ds(0, head), read_sems.at[n - 1]),
                part(pl.ds(head, _READ_TAIL), read_sems.at[n]))

    def write(phase, first, count, strips, sem):
        return [
            pltpu.make_async_copy(
                buf.at[pl.ds(first, count), s],
                o_hbm.at[pl.ds(phase * n * slabs + first, count), s], sem)
            for s in strips
        ]

    def write_front(phase):
        return write(phase, 0, last, range(_SLAB), write_sems.at[0])

    def write_last(phase):
        head = _SLAB - _WRITE_TAIL
        return (write(phase, last, slabs, range(head), write_sems.at[1]),
                write(phase, last, slabs, range(head, _SLAB), write_sems.at[2]))

    def normalize(slot, group):
        base = slot * slabs

        def mean_of(fn):
            def body(i, acc):
                for s in range(_SLAB):
                    v = fn(buf[base + i, s].astype(jnp.float32))
                    parts = [v[:, j:j + _LANES] for j in range(0, width, _LANES)]
                    while len(parts) > len(acc):
                        half = len(parts) // 2
                        parts = [p + q for p, q in zip(parts[:half], parts[half:])]
                    acc = tuple(a + p for a, p in zip(acc, parts))
                return acc

            zero = jnp.zeros((_ROWS, _LANES), jnp.float32)
            acc = lax.fori_loop(0, slabs, body, (zero,) * 4)
            total = (acc[0] + acc[1]) + (acc[2] + acc[3])
            return jnp.sum(total, keepdims=True) * inv_count

        mean = mean_of(lambda v: v)
        var = mean_of(lambda v: (v - mean) * (v - mean))
        rstd = 1.0 / jnp.sqrt(var + _EPS)

        def apply(i, _):
            channel = group * cpg + i * ch_per_slab
            row = lax.shift_right_logical(channel, 7)
            col = channel & (_LANES - 1)
            for c in range(ch_per_slab):
                scale = rstd * gb[0, row, col + c]
                shift = gb[1, row, col + c]
                for s in range(c * strips_per_ch, (c + 1) * strips_per_ch):
                    v = buf[base + i, s].astype(jnp.float32)
                    buf[base + i, s] = ((v - mean) * scale + shift).astype(buf.dtype)

        lax.fori_loop(0, slabs, apply, None)

    params = (pltpu.make_async_copy(g_hbm, gb_raw.at[0], param_sems.at[0]),
              pltpu.make_async_copy(b_hbm, gb_raw.at[1], param_sems.at[1]))
    _start(params)
    read(0, 0).start()
    _wait(params)
    gb_f32[...] = gb_raw[...].astype(jnp.float32)
    to_smem = pltpu.make_async_copy(gb_f32, gb, param_sems.at[0])
    to_smem.start()
    _start([read(0, slot) for slot in range(1, n - 1)])
    _start(read_last(0))
    to_smem.wait()

    def run_phase(phase, _):
        def run_group(slot, _):
            @pl.when(slot < n - 1)
            def _():
                read(phase, slot).wait()

            @pl.when(slot == n - 1)
            def _():
                head, tail = read_last(phase)
                head.wait()
                _start(write_front(phase))
                tail.wait()

            normalize(slot, (phase * n + slot) & (_GROUPS - 1))

        lax.fori_loop(0, n, run_group, None)

        head, tail = write_last(phase)
        _start(head)
        _start(tail)
        _wait(write_front(phase))
        _wait(head)

        @pl.when(phase < phases - 1)
        def _():
            _start([read(phase + 1, slot) for slot in range(n - 1)])

        _wait(tail)

        @pl.when(phase < phases - 1)
        def _():
            _start(read_last(phase + 1))

    lax.fori_loop(0, phases, run_phase, None)


@jax.jit
def pallas_standalone__groupnorm__prompt_kernel(
    x: jax.Array,
    g: jax.Array,
    b: jax.Array,
):
    batch, channels, height, width = x.shape
    cpg = channels // _GROUPS
    strips_per_ch = height // _ROWS
    slabs = cpg * strips_per_ch // _SLAB
    assert height % _ROWS == 0 and _SLAB % strips_per_ch == 0
    assert slabs * _SLAB == cpg * strips_per_ch and _LANES % cpg == 0
    assert (batch * _GROUPS) % _PHASE_GROUPS == 0 and channels % _LANES == 0
    assert width % (4 * _LANES) == 0 and width & (width - 1) == 0

    view = (batch * _GROUPS * slabs, _SLAB, _ROWS, width)
    params = (2, channels // _LANES, _LANES)
    hbm = pl.BlockSpec(memory_space=pl.ANY)
    out = pl.pallas_call(
        functools.partial(_groupnorm_kernel, cpg=cpg, strips_per_ch=strips_per_ch),
        in_specs=[hbm, hbm, hbm],
        out_specs=hbm,
        out_shape=jax.ShapeDtypeStruct(view, x.dtype),
        scratch_shapes=[
            pltpu.VMEM((_PHASE_GROUPS * slabs,) + view[1:], x.dtype),
            pltpu.VMEM(params, g.dtype),
            pltpu.VMEM(params, jnp.float32),
            pltpu.SMEM(params, jnp.float32),
            pltpu.SemaphoreType.DMA((_PHASE_GROUPS + 1,)),
            pltpu.SemaphoreType.DMA((3,)),
            pltpu.SemaphoreType.DMA((2,)),
        ],
        compiler_params=pltpu.CompilerParams(vmem_limit_bytes=100 * 2**20),
    )(x.reshape(view), g.reshape(params[1:]), b.reshape(params[1:]))
    return out.reshape(x.shape)
```

```python
import functools

import jax
import jax.numpy as jnp
from jax import lax
import jax.experimental.pallas as pl
import jax.experimental.pallas.tpu as pltpu

_GROUPS = 32
_EPS = 1e-5
_LANES = 128
_ROWS = 8
_SLAB_LOG2 = 5
_SLAB = 1 << _SLAB_LOG2
_UNIT = 2
_MAX_UNITS = 11
_READ_AHEAD = 4
_TURN_STRIP = 29
_FIRST_WRITES = 8


def _groupnorm_kernel(x_hbm, g_hbm, b_hbm, o_hbm, buf, gb_raw, gb_f32, gb,
                      read_sems, write_sems, param_sems, *, cpg, strips_per_ch):
    width = buf.shape[-1]
    half = width // 2
    slabs = cpg * strips_per_ch // _SLAB
    unit_slabs = _UNIT * slabs
    max_units = buf.shape[0] // unit_slabs
    total_units = x_hbm.shape[0] // unit_slabs
    phases = pl.cdiv(total_units, max_units)
    inv_count = 1.0 / (slabs * _SLAB * _ROWS * width)

    def window(ref, unit, strip, side, first=0, count=unit_slabs):
        return ref.at[pl.ds(unit * unit_slabs + first, count), strip, :,
                      pl.ds(side * half, half)]

    def reads(unit0, slot, strip, side):
        sem = read_sems.at[strip & (_READ_AHEAD - 1), side]
        return [
            pltpu.make_async_copy(
                window(x_hbm, unit0 + slot, strip, side, first, count),
                window(buf, slot, strip, side, first, count), sem)
            for first, count in ((0, 1), (1, unit_slabs - 1))
        ]

    def start_read(*chunk):
        for priority, copy in enumerate(reads(*chunk)):
            copy.start(priority=priority)

    def wait_read(*chunk):
        for copy in reads(*chunk):
            copy.wait()

    def start_first_reads(unit0):
        for strip in range(_READ_AHEAD):
            for side in range(2):
                start_read(unit0, 0, strip, side)

    def write(unit0, slot, strip, side, sem):
        return pltpu.make_async_copy(
            window(buf, slot, strip, side),
            window(o_hbm, unit0 + slot, strip, side), sem)

    def start_writes(unit0, lo, hi):
        def body(i, _):
            for side in range(2):
                write(unit0, lax.shift_right_logical(i, _SLAB_LOG2),
                      i & (_SLAB - 1), side, write_sems.at[0]).start()

        lax.fori_loop(lo, hi, body, None)

    def accumulate(acc, v):
        parts = [v[:, j:j + _LANES] for j in range(0, v.shape[1], _LANES)]
        while len(parts) > len(acc):
            mid = len(parts) // 2
            parts = [p + q for p, q in zip(parts[:mid], parts[mid:])]
        return tuple(a + p for a, p in zip(acc, parts))

    def average(acc):
        return jnp.sum(acc[0] + acc[1], keepdims=True) * inv_count

    def sweep(unit0, units, slot, stats, *, load, center, apply):
        mean_center, mean_apply, rstd_apply = stats

        def advance_reads(strip, side):
            wait_read(unit0, slot, strip, side)
            ahead = strip + _READ_AHEAD
            ahead_slot = slot + lax.shift_right_logical(ahead, _SLAB_LOG2)
            if not apply:
                start_read(unit0, ahead_slot, ahead & (_SLAB - 1), side)
                return

            @pl.when(ahead_slot < units)
            def _():
                start_read(unit0, ahead_slot, ahead & (_SLAB - 1), side)

            if side == 1:
                @pl.when((slot == units - 1) & (strip == _TURN_STRIP))
                def _():
                    start_writes(unit0, 0, _FIRST_WRITES)

        def body(strip, carry):
            sums, squares = map(list, carry)
            for k in range(_UNIT):
                if load:
                    advance_reads(strip, k)
                for q in range(slabs):
                    slab = slot * unit_slabs + k * slabs + q
                    if load:
                        for j in range(_UNIT):
                            v = buf[slot * unit_slabs + j * slabs + q, strip, :,
                                    pl.ds(k * half, half)]
                            sums[j] = accumulate(sums[j], v.astype(jnp.float32))
                    if center:
                        v = buf[slab - unit_slabs, strip].astype(jnp.float32)
                        d = v - mean_center[k]
                        squares[k] = accumulate(squares[k], d * d)
                    if apply:
                        group = ((unit0 + slot - 2) * _UNIT + k) & (_GROUPS - 1)
                        channel = (group * cpg + q * (_SLAB // strips_per_ch)
                                   + lax.shift_right_logical(
                                       strip, strips_per_ch.bit_length() - 1))
                        row = lax.shift_right_logical(channel, 7)
                        col = channel & (_LANES - 1)
                        scale = rstd_apply[k] * gb[0, row, col]
                        v = buf[slab - 2 * unit_slabs, strip].astype(jnp.float32)
                        y = (v - mean_apply[k]) * scale + gb[1, row, col]
                        buf[slab - 2 * unit_slabs, strip] = y.astype(buf.dtype)
            return tuple(sums), tuple(squares)

        zeros = ((jnp.zeros((_ROWS, _LANES), jnp.float32),) * 2,) * _UNIT
        sums, squares = lax.fori_loop(
            0, _SLAB, body, (zeros if load else (), zeros if center else ()))
        if load:
            next_mean = tuple(average(acc) for acc in sums)
        else:
            next_mean = mean_center
        if center:
            rstd_apply = tuple(
                1.0 / jnp.sqrt(average(acc) + _EPS) for acc in squares)
        return next_mean, mean_center, rstd_apply

    start_first_reads(0)
    params = (pltpu.make_async_copy(g_hbm, gb_raw.at[0], param_sems.at[0]),
              pltpu.make_async_copy(b_hbm, gb_raw.at[1], param_sems.at[1]))
    for copy in params:
        copy.start()
    params_to_smem = pltpu.make_async_copy(gb_f32, gb, param_sems.at[2])

    def run_phase(phase, _):
        unit0 = phase * max_units
        units = jnp.minimum(max_units, total_units - unit0)
        run = functools.partial(sweep, unit0, units)

        unset = (jnp.zeros((1, 1), jnp.float32),) * _UNIT
        stats = run(0, (unset,) * 3, load=True, center=False, apply=False)

        @pl.when(phase == 0)
        def _():
            for copy in params:
                copy.wait()
            gb_f32[...] = gb_raw[...].astype(jnp.float32)
            params_to_smem.start()

        stats = run(1, stats, load=True, center=True, apply=False)

        @pl.when(phase == 0)
        def _():
            params_to_smem.wait()

        stats = lax.fori_loop(
            2, units,
            functools.partial(run, load=True, center=True, apply=True), stats)

        start_writes(unit0, _FIRST_WRITES, _SLAB)
        stats = run(units, stats, load=False, center=True, apply=True)
        start_writes(unit0, _SLAB, 2 * _SLAB)
        run(units + 1, stats, load=False, center=False, apply=True)
        start_writes(unit0, 2 * _SLAB, units * _SLAB - 1)
        last = [write(unit0, units - 1, _SLAB - 1, side, write_sems.at[side])
                for side in range(2)]
        for copy in last:
            copy.start()

        def wait_unit(slot, _):
            whole = buf.at[pl.ds(slot * unit_slabs, unit_slabs)]
            pltpu.make_async_copy(whole, whole, write_sems.at[0]).wait()

        lax.fori_loop(0, units - 1, wait_unit, None)
        rest = buf.at[pl.ds(0, unit_slabs), pl.ds(0, _SLAB - 1)]
        pltpu.make_async_copy(rest, rest, write_sems.at[0]).wait()
        last[0].wait()

        @pl.when(phase < phases - 1)
        def _():
            start_first_reads(unit0 + units)

        last[1].wait()

    lax.fori_loop(0, phases, run_phase, None)


@jax.jit
def pallas_standalone__groupnorm__prompt_kernel(
    x: jax.Array,
    g: jax.Array,
    b: jax.Array,
):
    batch, channels, height, width = x.shape
    cpg = channels // _GROUPS
    strips_per_ch = height // _ROWS
    slabs = cpg * strips_per_ch // _SLAB
    total_units = batch * _GROUPS // _UNIT
    assert height % _ROWS == 0 and _SLAB % strips_per_ch == 0
    assert slabs * _SLAB == cpg * strips_per_ch and channels % _LANES == 0
    assert width >= 4 * _LANES and width & (width - 1) == 0
    assert (total_units - 1) % _MAX_UNITS >= 3

    view = (batch * _GROUPS * slabs, _SLAB, _ROWS, width)
    params = (2, channels // _LANES, _LANES)
    hbm = pl.BlockSpec(memory_space=pl.ANY)
    out = pl.pallas_call(
        functools.partial(_groupnorm_kernel, cpg=cpg, strips_per_ch=strips_per_ch),
        in_specs=[hbm, hbm, hbm],
        out_specs=hbm,
        out_shape=jax.ShapeDtypeStruct(view, x.dtype),
        scratch_shapes=[
            pltpu.VMEM((_MAX_UNITS * _UNIT * slabs,) + view[1:], x.dtype),
            pltpu.VMEM(params, g.dtype),
            pltpu.VMEM(params, jnp.float32),
            pltpu.SMEM(params, jnp.float32),
            pltpu.SemaphoreType.DMA((_READ_AHEAD, 2)),
            pltpu.SemaphoreType.DMA((2,)),
            pltpu.SemaphoreType.DMA((3,)),
        ],
        compiler_params=pltpu.CompilerParams(vmem_limit_bytes=100 * 2**20),
    )(x.reshape(view), g.reshape(params[1:]), b.reshape(params[1:]))
    return out.reshape(x.shape)
```

```python
import functools

import jax
import jax.numpy as jnp
from jax import lax
import jax.experimental.pallas as pl
import jax.experimental.pallas.tpu as pltpu

_GROUPS = 32
_EPS = 1e-5
_LANES = 128
_ROWS = 8
_SLAB_LOG2 = 5
_SLAB = 1 << _SLAB_LOG2
_UNIT = 2
_MAX_UNITS = 11
_READ_PARTS = ((slice(0, 2), 0, 5), (slice(2, None), 1, 8))
_READ_RING = 4
_TURN_STRIP = 29
_FIRST_WRITES = 8


def _groupnorm_kernel(x_hbm, g_hbm, b_hbm, o_hbm, buf, gb_raw, gb_f32, gb,
                      read_sems, write_sems, param_sems, *, cpg, strips_per_ch):
    width = buf.shape[-1]
    half = width // 2
    slabs = cpg * strips_per_ch // _SLAB
    unit_slabs = _UNIT * slabs
    max_units = buf.shape[0] // unit_slabs
    total_units = x_hbm.shape[0] // unit_slabs
    phases = pl.cdiv(total_units, max_units)
    inv_count = 1.0 / (slabs * _SLAB * _ROWS * width)

    def window(ref, unit, strip, side, part=slice(None)):
        first, end, _ = part.indices(unit_slabs)
        return ref.at[pl.ds(unit * unit_slabs + first, end - first), strip, :,
                      pl.ds(side * half, half)]

    def read(unit0, slot, strip, side, part):
        return pltpu.make_async_copy(
            window(x_hbm, unit0 + slot, strip, side, part),
            window(buf, slot, strip, side, part),
            read_sems.at[strip & (_READ_RING - 1), side])

    def start_first_reads(unit0):
        for chunk in range(2 * _READ_RING):
            for part, priority, ahead in _READ_PARTS:
                if chunk < ahead:
                    read(unit0, 0, *divmod(chunk, 2), part).start(priority=priority)

    def write(unit0, slot, strip, side, sem):
        return pltpu.make_async_copy(
            window(buf, slot, strip, side),
            window(o_hbm, unit0 + slot, strip, side), sem)

    def start_writes(unit0, lo, hi):
        def body(i, _):
            slot = lax.shift_right_logical(i, _SLAB_LOG2)
            for side in range(2):
                write(unit0, slot, i & (_SLAB - 1), side,
                      write_sems.at[slot]).start()

        lax.fori_loop(lo, hi, body, None)

    def accumulate(acc, v):
        parts = [v[:, j:j + _LANES] for j in range(0, v.shape[1], _LANES)]
        while len(parts) > len(acc):
            mid = len(parts) // 2
            parts = [p + q for p, q in zip(parts[:mid], parts[mid:])]
        return tuple(a + p for a, p in zip(acc, parts))

    def average(acc):
        return jnp.sum(acc[0] + acc[1], keepdims=True) * inv_count

    def sweep(unit0, units, slot, stats, *, load, center, apply):
        mean_center, mean_apply, rstd_apply = stats

        def advance_reads(strip, side):
            for part, _, _ in _READ_PARTS:
                read(unit0, slot, strip, side, part).wait()
            for part, priority, ahead in _READ_PARTS:
                skip, next_side = divmod(side + ahead, 2)
                next_slot = slot + lax.shift_right_logical(strip + skip, _SLAB_LOG2)

                def start():
                    read(unit0, next_slot, (strip + skip) & (_SLAB - 1),
                         next_side, part).start(priority=priority)

                if apply:
                    pl.when(next_slot < units)(start)
                else:
                    start()

            if apply and side == 1:
                @pl.when((slot == units - 1) & (strip == _TURN_STRIP))
                def _():
                    start_writes(unit0, 0, _FIRST_WRITES)

        def body(strip, carry):
            sums, squares = map(list, carry)
            for k in range(_UNIT):
                if load:
                    advance_reads(strip, k)
                for q in range(slabs):
                    slab = slot * unit_slabs + k * slabs + q
                    if load:
                        for j in range(_UNIT):
                            v = buf[slot * unit_slabs + j * slabs + q, strip, :,
                                    pl.ds(k * half, half)]
                            sums[j] = accumulate(sums[j], v.astype(jnp.float32))
                    if center:
                        v = buf[slab - unit_slabs, strip].astype(jnp.float32)
                        d = v - mean_center[k]
                        squares[k] = accumulate(squares[k], d * d)
                    if apply:
                        group = ((unit0 + slot - 2) * _UNIT + k) & (_GROUPS - 1)
                        channel = (group * cpg + q * (_SLAB // strips_per_ch)
                                   + lax.shift_right_logical(
                                       strip, strips_per_ch.bit_length() - 1))
                        row = lax.shift_right_logical(channel, 7)
                        col = channel & (_LANES - 1)
                        scale = rstd_apply[k] * gb[0, row, col]
                        v = buf[slab - 2 * unit_slabs, strip].astype(jnp.float32)
                        y = (v - mean_apply[k]) * scale + gb[1, row, col]
                        buf[slab - 2 * unit_slabs, strip] = y.astype(buf.dtype)
            return tuple(sums), tuple(squares)

        zeros = ((jnp.zeros((_ROWS, _LANES), jnp.float32),) * 2,) * _UNIT
        sums, squares = lax.fori_loop(
            0, _SLAB, body, (zeros if load else (), zeros if center else ()))
        if load:
            next_mean = tuple(average(acc) for acc in sums)
        else:
            next_mean = mean_center
        if center:
            rstd_apply = tuple(
                1.0 / jnp.sqrt(average(acc) + _EPS) for acc in squares)
        return next_mean, mean_center, rstd_apply

    start_first_reads(0)
    params = (pltpu.make_async_copy(g_hbm, gb_raw.at[0], param_sems.at[0]),
              pltpu.make_async_copy(b_hbm, gb_raw.at[1], param_sems.at[1]))
    for copy in params:
        copy.start()
    params_to_smem = pltpu.make_async_copy(gb_f32, gb, param_sems.at[2])

    def run_phase(phase, _):
        unit0 = phase * max_units
        units = jnp.minimum(max_units, total_units - unit0)
        run = functools.partial(sweep, unit0, units)

        unset = (jnp.zeros((1, 1), jnp.float32),) * _UNIT
        stats = run(0, (unset,) * 3, load=True, center=False, apply=False)

        @pl.when(phase == 0)
        def _():
            for copy in params:
                copy.wait()
            gb_f32[...] = gb_raw[...].astype(jnp.float32)
            params_to_smem.start()

        stats = run(1, stats, load=True, center=True, apply=False)

        @pl.when(phase == 0)
        def _():
            params_to_smem.wait()

        stats = lax.fori_loop(
            2, units,
            functools.partial(run, load=True, center=True, apply=True), stats)

        start_writes(unit0, _FIRST_WRITES, _SLAB)
        stats = run(units, stats, load=False, center=True, apply=True)
        start_writes(unit0, _SLAB, 2 * _SLAB)
        run(units + 1, stats, load=False, center=False, apply=True)
        start_writes(unit0, 2 * _SLAB, units * _SLAB - 1)
        last = [write(unit0, units - 1, _SLAB - 1, side,
                      write_sems.at[max_units + side]) for side in range(2)]
        for copy in last:
            copy.start()

        def wait_writes(slot, strips):
            done = buf.at[pl.ds(slot * unit_slabs, unit_slabs), pl.ds(0, strips)]
            pltpu.make_async_copy(done, done, write_sems.at[slot]).wait()

        lax.fori_loop(0, units - 1, lambda slot, _: wait_writes(slot, _SLAB), None)
        wait_writes(units - 1, _SLAB - 1)
        last[0].wait()

        @pl.when(phase < phases - 1)
        def _():
            start_first_reads(unit0 + units)

        last[1].wait()

    lax.fori_loop(0, phases, run_phase, None)


@jax.jit
def pallas_standalone__groupnorm__prompt_kernel(
    x: jax.Array,
    g: jax.Array,
    b: jax.Array,
):
    batch, channels, height, width = x.shape
    cpg = channels // _GROUPS
    strips_per_ch = height // _ROWS
    slabs = cpg * strips_per_ch // _SLAB
    total_units = batch * _GROUPS // _UNIT
    assert height % _ROWS == 0 and _SLAB % strips_per_ch == 0
    assert slabs * _SLAB == cpg * strips_per_ch and channels % _LANES == 0
    assert width >= 4 * _LANES and width & (width - 1) == 0
    assert (total_units - 1) % _MAX_UNITS >= 3

    view = (batch * _GROUPS * slabs, _SLAB, _ROWS, width)
    params = (2, channels // _LANES, _LANES)
    hbm = pl.BlockSpec(memory_space=pl.ANY)
    out = pl.pallas_call(
        functools.partial(_groupnorm_kernel, cpg=cpg, strips_per_ch=strips_per_ch),
        in_specs=[hbm, hbm, hbm],
        out_specs=hbm,
        out_shape=jax.ShapeDtypeStruct(view, x.dtype),
        scratch_shapes=[
            pltpu.VMEM((_MAX_UNITS * _UNIT * slabs,) + view[1:], x.dtype),
            pltpu.VMEM(params, g.dtype),
            pltpu.VMEM(params, jnp.float32),
            pltpu.SMEM(params, jnp.float32),
            pltpu.SemaphoreType.DMA((_READ_RING, 2)),
            pltpu.SemaphoreType.DMA((_MAX_UNITS + 2,)),
            pltpu.SemaphoreType.DMA((3,)),
        ],
        compiler_params=pltpu.CompilerParams(
            vmem_limit_bytes=100 * 2**20,
            disable_bounds_checks=True,
            disable_semaphore_checks=True),
    )(x.reshape(view), g.reshape(params[1:]), b.reshape(params[1:]))
    return out.reshape(x.shape)
```
